```python
import os as _os
_os.environ.setdefault("JAX_PLATFORMS", "cpu")
import jax
import jax.numpy as jnp

def _softmax(x, axis=-1):
    return jax.nn.softmax(x, axis=axis)
def _gelu(x):
    return jax.nn.gelu(x, approximate=True)
def _silu(x):
    return jax.nn.silu(x)
def _sigmoid(x):
    return jax.nn.sigmoid(x)
def _layernorm(x, axis=-1, eps=1e-5):
    m = jnp.mean(x, axis=axis, keepdims=True)
    v = jnp.var(x, axis=axis, keepdims=True)
    return (x - m) / jnp.sqrt(v + eps)
def _scatter_add(tgt, idx, src, axis=0):
    return tgt.at[idx].add(src)
def _segment_sum(src, seg, n):
    return jax.ops.segment_sum(src, seg, n)
class _Rng:
    def __init__(self, key):
        self._k = key
    def _next(self):
        self._k, sub = jax.random.split(self._k)
        return sub
    def normal(self, shape):
        return jax.random.normal(self._next(), shape, dtype=jnp.bfloat16)
    def randint(self, lo, hi, shape):
        return jax.random.randint(self._next(), shape, lo, hi, dtype=jnp.int32)
    def uniform(self, shape, lo=0.0, hi=1.0):
        return jax.random.uniform(self._next(), shape, jnp.bfloat16, lo, hi)
    def permutation(self, n):
        return jax.random.permutation(self._next(), n)


kernel_name = 'concat_heads__gqa_block_cached__sliding_block_cached__decode'

def setup_inputs():
    _rng = _Rng(jax.random.key(int.from_bytes(__import__("os").urandom(4), "little")))
    _w = (lambda a: (lambda t: t.astype(jnp.bfloat16) if jnp.issubdtype(t.dtype, jnp.floating) else t)(jnp.asarray(a)))
    def _A_setup():
        B, Sq, D = 1, 1, 576
        Hq, Hkv, Sk, Dh = 32, 16, 8192, 128
        assert Hq % Hkv == 0, (Hq, Hkv)
        return {
            "x": _w((lambda *s: _rng.normal(s) * 0.8)(B, Sq, D)),
            "k_cache": _w((lambda *s: _rng.normal(s) * 0.8)(B, Hkv, Sk, Dh)),
            "v_cache": _w((lambda *s: _rng.normal(s) * 0.05)(B, Hkv, Sk, Dh)),
            "wq": _w((lambda *s: _rng.normal(s) * 0.8)(D, Hq * Dh) * (D ** -0.5)),
            "wo": _w((lambda *s: _rng.normal(s) * 0.05)(Hq * Dh, D) * ((Hq * Dh) ** -0.5)),
        }
    _A_in = _A_setup()

    def _B_setup():
        B, Sq, D = 1, 1, 576
        Hq, Hkv, Sk, Dh = 32, 16, 8192, 128
        assert Hq % Hkv == 0, (Hq, Hkv)
        return {
            "x": _w((lambda *s: _rng.normal(s) * 0.8)(B, Sq, D)),
            "k_cache": _w((lambda *s: _rng.normal(s) * 0.8)(B, Hkv, Sk, Dh)),
            "v_cache": _w((lambda *s: _rng.normal(s) * 0.05)(B, Hkv, Sk, Dh)),
            "wq": _w((lambda *s: _rng.normal(s) * 0.8)(D, Hq * Dh) * (D ** -0.5)),
            "wo": _w((lambda *s: _rng.normal(s) * 0.05)(Hq * Dh, D) * ((Hq * Dh) ** -0.5)),
        }
    _B_in = _B_setup()

    return {
        "A_x": _A_in["x"],
        "A_k_cache": _A_in["k_cache"],
        "A_v_cache": _A_in["v_cache"],
        "A_wq": _A_in["wq"],
        "A_wo": _A_in["wo"],
        "B_x": _B_in["x"],
        "B_k_cache": _B_in["k_cache"],
        "B_v_cache": _B_in["v_cache"],
        "B_wq": _B_in["wq"],
        "B_wo": _B_in["wo"],
    }

def reference(A_x, A_k_cache, A_v_cache, A_wq, A_wo, B_x, B_k_cache, B_v_cache, B_wq, B_wo):
    def _A_ref(x, k_cache, v_cache, wq, wo):
        B, Sq, D = x.shape
        Hq, Dh = 32, 128
        Hkv = k_cache.shape[1]
        rep = Hq // Hkv
        q = (lambda x, *d: x.transpose(*d))((x @ wq).reshape(B, Sq, Hq, Dh), 0, 2, 1, 3)
        k = jnp.repeat(k_cache, rep, axis=1)
        v = jnp.repeat(v_cache, rep, axis=1)
        scores = jnp.einsum("bhqd,bhkd->bhqk", q, k) * (Dh ** -0.5)
        p = _softmax(scores, axis=-1)
        o = jnp.einsum("bhqk,bhkd->bhqd", p, v)
        return (lambda x, *d: x.transpose(*d))(o, 0, 2, 1, 3).reshape(B, Sq, Hq * Dh) @ wo

    def _B_ref(x, k_cache, v_cache, wq, wo):
        B, Sq, D = x.shape
        Hq, Dh = 32, 128
        Hkv, Sk = k_cache.shape[1], k_cache.shape[2]
        W = min(4096, max(256, Sk // 4))
        rep = Hq // Hkv
        q = (lambda x, *d: x.transpose(*d))((x @ wq).reshape(B, Sq, Hq, Dh), 0, 2, 1, 3)
        k = jnp.repeat(k_cache[:, :, Sk - W:, :], rep, axis=1)
        v = jnp.repeat(v_cache[:, :, Sk - W:, :], rep, axis=1)
        scores = jnp.einsum("bhqd,bhkd->bhqk", q, k) * (Dh ** -0.5)
        p = _softmax(scores, axis=-1)
        o = jnp.einsum("bhqk,bhkd->bhqd", p, v)
        return (lambda x, *d: x.transpose(*d))(o, 0, 2, 1, 3).reshape(B, Sq, Hq * Dh) @ wo

    a = _A_ref(A_x, A_k_cache, A_v_cache, A_wq, A_wo)
    b = _B_ref(B_x, B_k_cache, B_v_cache, B_wq, B_wo)
    return jnp.concatenate([a, b], axis=-1)
```

```python
import functools
import jax
import jax.numpy as jnp
import numpy as np
from jax import lax
from jax.experimental import pallas as pl
from jax.experimental.pallas import tpu as pltpu

HQ, DH = 32, 128
TILE = 128
HG = 4
NT = (((1,), (1,)), ((), ()))


def make(step_rows=512, look=4, wrows=8, nobc=True, nosem=True, extra_slot=0, compute=True):
    def kernel(xa, ka, va, wqa, woa, xb, kb, vb, wqb, wob, out_ref,
               x_buf, wq_buf, wo_buf, kv_buf, o_buf, w_sem, kv_sem):
        d_model = wqa.shape[0]
        hkv, sk = ka.shape[1], ka.shape[2]
        win = min(4096, max(256, sk // 4))
        ngrp = hkv // HG
        spa, spb = sk // step_rows, win // step_rows
        na, nb = ngrp * spa, ngrp * spb
        nslot = look + extra_slot
        wcols = 16384 // wrows
        cper = HQ * DH // wcols
        nw = d_model // wrows * cper
        rper = d_model // wrows // 4

        def start_weights(a, b, dst_a, dst_b, sem):
            def body(i, c):
                for cc in range(cper):
                    for t in range(4):
                        r = pl.ds(pl.multiple_of((t * rper + i) * wrows, wrows), wrows)
                        cs = pl.ds(cc * wcols, wcols)
                        pltpu.make_async_copy(b.at[r, cs], dst_b.at[r, cs], sem).start(priority=1)
                        pltpu.make_async_copy(a.at[r, cs], dst_a.at[r, cs], sem).start(priority=0)
                return c
            lax.fori_loop(0, rper, body, 0)

        def start_kv(k, v, grp, row0, slot):
            for t in range(step_rows // TILE):
                r = pl.ds(pl.multiple_of(row0 + t * TILE, TILE), TILE)
                rd = pl.ds(t * TILE, TILE)
                for j in range(HG):
                    h = grp * HG + j
                    pltpu.make_async_copy(v.at[0, h, r, :], kv_buf.at[slot, 1, j, rd, :], kv_sem.at[slot]).start(priority=1)
                    pltpu.make_async_copy(k.at[0, h, r, :], kv_buf.at[slot, 0, j, rd, :], kv_sem.at[slot]).start(priority=0)

        def start_step(s):
            slot = s % nslot

            @pl.when(s < na)
            def _():
                start_kv(ka, va, s // spa, (s % spa) * step_rows, slot)

            @pl.when(jnp.logical_and(s >= na, s < na + nb))
            def _():
                u = s - na
                start_kv(kb, vb, u // spb, sk - win + (u % spb) * step_rows, slot)

            @pl.when(s == na + nb)
            def _():
                start_weights(woa, wob, wo_buf.at[pl.ds(0, d_model)], wo_buf.at[pl.ds(d_model, d_model)], w_sem.at[0])

        x_copies = [pltpu.make_async_copy(x.at[0], x_buf.at[i], w_sem.at[1]) for i, x in enumerate((xa, xb))]
        start_weights(wqa, wqb, wq_buf.at[0], wq_buf.at[1], w_sem.at[0])
        for c in x_copies:
            c.start()
        lax.fori_loop(0, look, lambda s, c: (start_kv(ka, va, s // spa, (s % spa) * step_rows, s), c)[1], 0)
        for c in x_copies:
            c.wait()
        pltpu.make_async_copy(wq_buf, wq_buf, w_sem.at[0]).wait()

        row = lax.broadcasted_iota(jnp.int32, (8, DH), 0)
        scale = np.float32(DH ** -0.5)

        def group(gi, s0):
            br = gi // ngrp
            g = gi % ngrp
            x = jnp.broadcast_to(x_buf[br], (8, d_model))
            cols = pl.ds(pl.multiple_of(g * 8 * DH, 8 * DH), 8 * DH)
            qf = jnp.dot(x, wq_buf[br, :, cols], preferred_element_type=jnp.float32)
            q = qf[:, :DH]
            for r in range(1, 8):
                q = jnp.where(row == r, qf[:, r * DH:(r + 1) * DH], q)
            q = q.astype(jnp.bfloat16)

            def step(s, carry):
                m, l, acc = carry
                slot = s % nslot
                pltpu.make_async_copy(kv_buf.at[slot], kv_buf.at[slot], kv_sem.at[slot]).wait()
                if extra_slot:
                    start_step(s + look)
                if compute:
                    rows = lax.broadcasted_iota(jnp.int32, (8, step_rows), 0)
                    sc = None
                    for j in range(HG):
                        sj = lax.dot_general(q, kv_buf[slot, 0, j], NT, preferred_element_type=jnp.float32)
                        sc = sj if j == 0 else jnp.where(rows >= 2 * j, sj, sc)
                    sc = sc * scale
                    m_new = jnp.maximum(m, jnp.max(sc, axis=1, keepdims=True))
                    alpha = jnp.exp(m - m_new)
                    p = jnp.exp(sc - m_new[:, :1])
                    ps = p[:, :DH]
                    for t in range(1, step_rows // DH):
                        ps = ps + p[:, t * DH:(t + 1) * DH]
                    pb = p.astype(jnp.bfloat16)
                    pv = None
                    for j in range(HG):
                        oj = jnp.dot(pb, kv_buf[slot, 1, j], preferred_element_type=jnp.float32)
                        pv = oj if j == 0 else jnp.where(row >= 2 * j, oj, pv)
                    m, l, acc = m_new, alpha * l + ps, alpha * acc + pv
                if not extra_slot:
                    start_step(s + look)
                return m, l, acc

            s1 = s0 + jnp.where(br == 0, spa, spb)
            init = (jnp.full((8, DH), np.finfo(np.float32).min, jnp.float32),
                    jnp.zeros((8, DH), jnp.float32), jnp.zeros((8, DH), jnp.float32))
            m, l, acc = lax.fori_loop(s0, s1, step, init)
            o = acc / jnp.sum(l, axis=1, keepdims=True)
            ob = jnp.concatenate([jnp.broadcast_to(o[r:r + 1], (8, DH)) for r in range(8)], axis=1)
            o_buf[br, :, cols] = ob
            return s1

        lax.fori_loop(0, 2 * ngrp, group, 0)

        pltpu.make_async_copy(wo_buf, wo_buf, w_sem.at[0]).wait()
        lhs = o_buf[...].reshape(16, HQ * DH).astype(jnp.bfloat16)
        res = lax.dot_general(lhs, wo_buf[...], NT, preferred_element_type=jnp.float32)
        col = lax.broadcasted_iota(jnp.int32, (8, 2 * d_model), 1)
        res = jnp.where(col < d_model, res[:8], res[8:])
        out_ref[0] = res[:1].astype(out_ref.dtype)

    def fn(A_x, A_k, A_v, A_wq, A_wo, B_x, B_k, B_v, B_wq, B_wo):
        d_model = A_wq.shape[0]
        hbm = pl.BlockSpec(memory_space=pltpu.HBM)
        return pl.pallas_call(
            kernel,
            in_specs=[hbm] * 10,
            out_specs=pl.BlockSpec(memory_space=pltpu.VMEM),
            out_shape=jax.ShapeDtypeStruct((1, 1, 2 * d_model), A_x.dtype),
            scratch_shapes=[
                pltpu.VMEM((2, 1, d_model), jnp.bfloat16),
                pltpu.VMEM((2, d_model, HQ * DH), jnp.bfloat16),
                pltpu.VMEM((2 * d_model, HQ * DH), jnp.bfloat16),
                pltpu.VMEM((look + extra_slot, 2, HG, step_rows, DH), jnp.bfloat16),
                pltpu.VMEM((2, 8, HQ * DH), jnp.float32),
                pltpu.SemaphoreType.DMA((2,)),
                pltpu.SemaphoreType.DMA((look + extra_slot,)),
            ],
            compiler_params=pltpu.CompilerParams(
                vmem_limit_bytes=64 * 2**20, disable_bounds_checks=nobc, disable_semaphore_checks=nosem),
        )(A_x, A_k, A_v, A_wq, A_wo.T, B_x, B_k, B_v, B_wq, B_wo.T)
    return fn


@jax.jit
def pallas_concat_heads__gqa_block_cached__sliding_block_cached__decode_kernel(
    A_x, A_k_cache, A_v_cache, A_wq, A_wo, B_x, B_k_cache, B_v_cache, B_wq, B_wo,
):
    return make()(A_x, A_k_cache, A_v_cache, A_wq, A_wo, B_x, B_k_cache, B_v_cache, B_wq, B_wo)
```

```python
import jax
import jax.experimental.pallas as pl
import jax.experimental.pallas.tpu as pltpu
import jax.numpy as jnp
import numpy as np
from jax import lax

HQ, DH = 32, 128

KV_GROUP = 8
Q_GROUP = 16
STEP = 256
SLOTS = 4
KV_PIECE = 64

W_ROWS, W_COLS = 8, 1024
BAND = 64
BAND_ORDER = (0, 2, 4, 6, 8, 1, 3, 5, 7)
TAIL_CUTS = (768, 1024, 1152)

HIGH, LOW = 0, 1
_NT = (((1,), (1,)), ((), ()))


def _ds(start, size):
    if isinstance(start, int):
        return pl.ds(start, size)
    return pl.ds(pl.multiple_of(start, size), size)


def _wait_filled(buf, sem):
    pltpu.make_async_copy(buf, buf, sem).wait()


def _weight_copies(src, dst, sem, *positions):
    copies = []
    for row_group, col_block in positions:
        for band in BAND_ORDER:
            idx = (
                _ds(band * BAND + row_group * W_ROWS, W_ROWS),
                _ds(col_block * W_COLS, W_COLS),
            )
            copies.append(pltpu.make_async_copy(src.at[idx], dst.at[idx], sem))
    return copies


def _start_in_turns(low, high, low_turn=2):
    for i in range(len(low) // low_turn):
        for copy in low[low_turn * i : low_turn * (i + 1)]:
            copy.start(priority=LOW)
        for copy in high[2 * i : 2 * i + 2]:
            copy.start(priority=HIGH)


def _kernel(
    xa, ka, va, wqa, woa, xb, kb, vb, wqb, wob,
    out_ref,
    x_buf, wq_buf, wo_buf, kv_buf, o_buf, w_sem, kv_sem,
):
    d_model = wqa.shape[0]
    hkv, sk = ka.shape[1], ka.shape[2]
    window = min(4096, max(256, sk // 4))
    groups = hkv // KV_GROUP
    rep = HQ // hkv
    steps_a, steps_b = sk // STEP, window // STEP
    end_a = groups * steps_a
    end_b = end_a + groups * steps_b
    row_groups = BAND // W_ROWS
    wo_buf_a = wo_buf.at[pl.ds(0, d_model)]
    wo_buf_b = wo_buf.at[pl.ds(d_model, d_model)]

    def wq_copies(branch, n):
        src = (wqa, wqb)[branch]
        col = 2 * (n % 2)
        return _weight_copies(
            src, wq_buf.at[branch], w_sem.at[0], (n // 2, col), (n // 2, col + 1)
        )

    def start_wo(sem, *positions):
        _start_in_turns(
            _weight_copies(wob, wo_buf_b, sem, *positions),
            _weight_copies(woa, wo_buf_a, sem, *positions),
        )

    def start_kv(k, v, group, key0, slot):
        @pl.loop(0, STEP // KV_PIECE)
        def _(t):
            keys = _ds(key0 + t * KV_PIECE, KV_PIECE)
            for j in range(0, KV_GROUP, 2):
                heads = pl.ds(group * KV_GROUP + j, 2)
                for src, is_v, priority in ((v, 1, LOW), (k, 0, HIGH)):
                    pltpu.make_async_copy(
                        src.at[0, heads, keys, :],
                        kv_buf.at[slot, is_v, pl.ds(j, 2), _ds(t * KV_PIECE, KV_PIECE), :],
                        kv_sem.at[slot],
                    ).start(priority=priority)

    def start_step(s):
        slot = s % SLOTS

        @pl.when(s < end_a)
        def _():
            start_kv(ka, va, s // steps_a, (s % steps_a) * STEP, slot)

        @pl.when(jnp.logical_and(s >= end_a, s < end_b))
        def _():
            u = s - end_a
            start_kv(kb, vb, u // steps_b, sk - window + (u % steps_b) * STEP, slot)

        @pl.when(s >= end_b)
        def _():
            per_step = row_groups // SLOTS

            @pl.loop((s - end_b) * per_step, (s - end_b + 1) * per_step)
            def _(n):
                start_wo(w_sem.at[0], (n, 0), (n, 1))

    lead = 2
    wq_parts = 2 * row_groups

    @pl.loop(0, lead)
    def _(n):
        _start_in_turns(wq_copies(1, n), [])

    @pl.loop(0, wq_parts - lead)
    def _(n):
        _start_in_turns(wq_copies(1, n + lead), wq_copies(0, n))

    _start_in_turns(wq_copies(0, wq_parts - 1), wq_copies(0, wq_parts - 2))

    x_copies = [
        pltpu.make_async_copy(x.at[0], x_buf.at[i], w_sem.at[1])
        for i, x in enumerate((xa, xb))
    ]
    for copy in x_copies:
        copy.start()

    @pl.loop(0, SLOTS)
    def _(s):
        start_kv(ka, va, 0, s * STEP, s)

    for copy in x_copies:
        copy.wait()
    _wait_filled(wq_buf, w_sem.at[0])

    row = lax.broadcasted_iota(jnp.int32, (Q_GROUP, DH), 0)
    scale = np.float32(DH**-0.5)

    def attend_group(i, first_step):
        branch, group = i // groups, i % groups
        cols = _ds(group * Q_GROUP * DH, Q_GROUP * DH)
        x = jnp.broadcast_to(x_buf[branch], (Q_GROUP, d_model))
        q_all = jnp.dot(x, wq_buf[branch, :, cols], preferred_element_type=jnp.float32)
        q = q_all[:, :DH]
        for r in range(1, Q_GROUP):
            q = jnp.where(row == r, q_all[:, r * DH : (r + 1) * DH], q)
        q = q.astype(kv_buf.dtype)

        def step(s, carry):
            m, l, acc = carry
            slot = s % SLOTS
            _wait_filled(kv_buf.at[slot], kv_sem.at[slot])
            score_row = lax.broadcasted_iota(jnp.int32, (Q_GROUP, STEP), 0)
            scores = None
            for j in range(KV_GROUP):
                s_j = lax.dot_general(
                    q, kv_buf[slot, 0, j], _NT, preferred_element_type=jnp.float32
                )
                scores = s_j if j == 0 else jnp.where(score_row >= rep * j, s_j, scores)
            scores = scores * scale
            m_new = jnp.maximum(m, jnp.max(scores, axis=1, keepdims=True))
            alpha = jnp.exp(m - m_new)
            p = jnp.exp(scores - m_new[:, :1])
            p_sum = p[:, :DH]
            for t in range(1, STEP // DH):
                p_sum = p_sum + p[:, t * DH : (t + 1) * DH]
            p = p.astype(kv_buf.dtype)
            pv = None
            for j in range(KV_GROUP):
                pv_j = jnp.dot(p, kv_buf[slot, 1, j], preferred_element_type=jnp.float32)
                pv = pv_j if j == 0 else jnp.where(row >= rep * j, pv_j, pv)
            start_step(s + SLOTS)
            return m_new, alpha * l + p_sum, alpha * acc + pv

        last_step = first_step + jnp.where(branch == 0, steps_a, steps_b)
        zeros = jnp.zeros((Q_GROUP, DH), jnp.float32)
        m0 = jnp.full((Q_GROUP, DH), np.finfo(np.float32).min, jnp.float32)
        _, l, acc = lax.fori_loop(first_step, last_step, step, (m0, zeros, zeros))
        o = acc / jnp.sum(l, axis=1, keepdims=True)
        o_buf[branch, :, cols] = jnp.concatenate(
            [jnp.broadcast_to(o[r : r + 1], (8, DH)) for r in range(Q_GROUP)], axis=1
        )
        return last_step

    lax.fori_loop(0, 2 * groups, attend_group, 0)

    def project(rows, col_block):
        cols = _ds(col_block * W_COLS, W_COLS)
        o = o_buf[:, :, cols].reshape(16, W_COLS).astype(wo_buf.dtype)
        return lax.dot_general(
            o, wo_buf[rows, cols], _NT, preferred_element_type=jnp.float32
        )

    def start_wo_tail():
        cols = _ds(3 * W_COLS, W_COLS)
        low = []
        for r in range(0, d_model, 2 * W_ROWS):
            part = sum(d_model + r >= cut for cut in TAIL_CUTS)
            rows = _ds(r, 2 * W_ROWS)
            low.append(
                pltpu.make_async_copy(
                    wob.at[rows, cols], wo_buf_b.at[rows, cols], kv_sem.at[part]
                )
            )
        high = _weight_copies(
            woa, wo_buf_a, kv_sem.at[0], *[(n, 3) for n in range(row_groups)]
        )
        _start_in_turns(low, high, low_turn=1)

    @pl.loop(0, row_groups // 2)
    def _(n):
        start_wo(w_sem.at[1], (2 * n, 2), (2 * n + 1, 2))

    _wait_filled(wo_buf.at[:, pl.ds(0, 2 * W_COLS)], w_sem.at[0])

    def project_block(col_block, out):
        pl.when(col_block == 1)(start_wo_tail)

        @pl.when(col_block == 2)
        def _():
            _wait_filled(wo_buf.at[:, pl.ds(2 * W_COLS, W_COLS)], w_sem.at[1])

        return out + project(slice(None), col_block)

    out = lax.fori_loop(0, 3, project_block, jnp.zeros((16, 2 * d_model), jnp.float32))

    for part, (lo, hi) in enumerate(zip((0,) + TAIL_CUTS[:-1], TAIL_CUTS)):
        rows = pl.ds(lo, hi - lo)
        _wait_filled(wo_buf.at[rows, pl.ds(3 * W_COLS, W_COLS)], kv_sem.at[part])
        both = out[:, lo:hi] + project(rows, 3)
        result = both[8:]
        if lo < d_model:
            col = lo + lax.broadcasted_iota(jnp.int32, result.shape, 1)
            result = jnp.where(col < d_model, both[:8], result)
        out_ref[0, :, lo:hi] = result[:1].astype(out_ref.dtype)


@jax.jit
def pallas_concat_heads__gqa_block_cached__sliding_block_cached__decode_kernel(
    A_x: jax.Array,
    A_k_cache: jax.Array,
    A_v_cache: jax.Array,
    A_wq: jax.Array,
    A_wo: jax.Array,
    B_x: jax.Array,
    B_k_cache: jax.Array,
    B_v_cache: jax.Array,
    B_wq: jax.Array,
    B_wo: jax.Array,
):
    d_model = BAND * len(BAND_ORDER)
    assert A_x.shape == B_x.shape == (1, 1, d_model)
    assert A_wq.shape == B_wq.shape == (d_model, 4 * W_COLS)
    assert A_k_cache.shape == B_k_cache.shape
    assert A_k_cache.shape[1] * Q_GROUP == HQ * KV_GROUP
    assert A_k_cache.shape[2] % (4 * STEP) == 0

    in_hbm = pl.BlockSpec(memory_space=pltpu.MemorySpace.HBM)
    return pl.pallas_call(
        _kernel,
        in_specs=[in_hbm] * 10,
        out_specs=pl.BlockSpec(memory_space=pltpu.MemorySpace.VMEM),
        out_shape=jax.ShapeDtypeStruct((1, 1, 2 * d_model), A_x.dtype),
        scratch_shapes=[
            pltpu.VMEM((2, 1, d_model), A_x.dtype),
            pltpu.VMEM((2, d_model, HQ * DH), A_wq.dtype),
            pltpu.VMEM((2 * d_model, HQ * DH), A_wo.dtype),
            pltpu.VMEM((SLOTS, 2, KV_GROUP, STEP, DH), A_k_cache.dtype),
            pltpu.VMEM((2, 8, HQ * DH), jnp.float32),
            pltpu.SemaphoreType.DMA((2,)),
            pltpu.SemaphoreType.DMA((SLOTS,)),
        ],
        compiler_params=pltpu.CompilerParams(
            vmem_limit_bytes=64 * 2**20,
            disable_bounds_checks=True,
            disable_semaphore_checks=True,
        ),
    )(A_x, A_k_cache, A_v_cache, A_wq, A_wo.T, B_x, B_k_cache, B_v_cache, B_wq, B_wo.T)
```
